```python
import os as _os
_os.environ.setdefault("JAX_PLATFORMS", "cpu")
import jax
import jax.numpy as jnp

def _softmax(x, axis=-1):
    return jax.nn.softmax(x, axis=axis)
def _gelu(x):
    return jax.nn.gelu(x, approximate=True)
def _silu(x):
    return jax.nn.silu(x)
def _sigmoid(x):
    return jax.nn.sigmoid(x)
def _layernorm(x, axis=-1, eps=1e-5):
    m = jnp.mean(x, axis=axis, keepdims=True)
    v = jnp.var(x, axis=axis, keepdims=True)
    return (x - m) / jnp.sqrt(v + eps)
def _scatter_add(tgt, idx, src, axis=0):
    return tgt.at[idx].add(src)
def _segment_sum(src, seg, n):
    return jax.ops.segment_sum(src, seg, n)
class _Rng:
    def __init__(self, key):
        self._k = key
    def _next(self):
        self._k, sub = jax.random.split(self._k)
        return sub
    def normal(self, shape):
        return jax.random.normal(self._next(), shape, dtype=jnp.bfloat16)
    def randint(self, lo, hi, shape):
        return jax.random.randint(self._next(), shape, lo, hi, dtype=jnp.int32)
    def uniform(self, shape, lo=0.0, hi=1.0):
        return jax.random.uniform(self._next(), shape, jnp.bfloat16, lo, hi)
    def permutation(self, n):
        return jax.random.permutation(self._next(), n)


kernel_name = 'standalone__grn__sampling'

def setup_inputs():
    _rng = _Rng(jax.random.key(int.from_bytes(__import__("os").urandom(4), "little")))
    _w = (lambda a: (lambda t: t.astype(jnp.bfloat16) if jnp.issubdtype(t.dtype, jnp.floating) else t)(jnp.asarray(a)))
    B, S, D = 512, 32, 640
    return {
        "x": _w((lambda *s: _rng.normal(s) * 0.05)(B, S, D)),
        "g": _w((lambda *s: _rng.normal(s) * 0.1)(D) * 0.1),
        "b": _w((lambda *s: _rng.normal(s) * 0.1)(D) * 0.1),
    }

def reference(x, g, b):
    gx = jnp.sqrt((x * x).sum(axis=-2, keepdims=True))
    nx = gx / (gx.mean(axis=-1, keepdims=True) + 1e-6)
    return g * (x * nx) + b + x
```

```python
import jax
import jax.numpy as jnp
import jax.experimental.pallas as pl
import jax.experimental.pallas.tpu as pltpu

_EPS = 1e-6
_G = 8
_L = 4
_TAIL = 2


def _grn_kernel(x_hbm, g_hbm, b_hbm, o_hbm, buf, gbuf, bbuf, gf, bf, part, scl,
                rsem, wsem, gbsem):
    G, M, S, D = x_hbm.shape
    NC = D // 128

    def start_read(m, slot):
        for g in range(G):
            pltpu.make_async_copy(x_hbm.at[g, m], buf.at[g, m], rsem.at[slot]).start(
                priority=g % 2)

    def wait_read(m, slot):
        pltpu.make_async_copy(x_hbm.at[:, m], buf.at[:, m], rsem.at[slot]).wait()

    def start_write(m):
        pltpu.make_async_copy(buf.at[:, m], o_hbm.at[:, m], wsem).start()

    start_read(0, 0)
    cg = pltpu.make_async_copy(g_hbm, gbuf, gbsem.at[0])
    cb = pltpu.make_async_copy(b_hbm, bbuf, gbsem.at[1])
    cg.start()
    cb.start()
    for m in range(1, _L):
        start_read(m, m)
    cg.wait()
    cb.wait()
    gf[...] = jnp.broadcast_to(gbuf[...].astype(jnp.float32).reshape(1, D), (G, D))
    bf[...] = jnp.broadcast_to(bbuf[...].astype(jnp.float32).reshape(1, D), (G, D))

    def compute(m):
        for g in range(G):
            x = buf[g, m].astype(jnp.float32)
            sq = x * x
            p = sq[0:8]
            for s in range(1, S // 8):
                p = p + sq[8 * s:8 * s + 8]
            for c in range(NC):
                part[c, pl.ds(8 * g, 8), :] = p[:, c * 128:(c + 1) * 128]
        gxs = []
        for c in range(NC):
            q = part[c, pl.ds(0, G, stride=8), :]
            for r in range(1, 8):
                q = q + part[c, pl.ds(r, G, stride=8), :]
            gxs.append(jnp.sqrt(q))
        tot = gxs[0]
        for c in range(1, NC):
            tot = tot + gxs[c]
        inv = 1.0 / (jnp.sum(tot, axis=-1, keepdims=True) * (1.0 / D) + _EPS)
        for c in range(NC):
            cs = slice(c * 128, (c + 1) * 128)
            scl[:, cs] = gf[:, cs] * (gxs[c] * inv) + 1.0
        for g in range(G):
            x = buf[g, m].astype(jnp.float32)
            sc = jnp.broadcast_to(scl[pl.ds(g, 1), :], (S, D))
            bb = jnp.broadcast_to(bf[pl.ds(0, 1), :], (S, D))
            buf[g, m] = (x * sc + bb).astype(buf.dtype)

    def body1(m, _):
        slot = jax.lax.rem(m, _L)
        wait_read(m, slot)
        start_read(m + _L, slot)
        compute(m)

    jax.lax.fori_loop(0, M - _L, body1, None)

    def body2(m, _):
        wait_read(m, jax.lax.rem(m, _L))

        @pl.when(m == M - 1 - _TAIL)
        def _():
            jax.lax.fori_loop(0, m, lambda i, _: start_write(i), None)

        compute(m)

        @pl.when(m >= M - 1 - _TAIL)
        def _():
            start_write(m)

    jax.lax.fori_loop(M - _L, M, body2, None)
    pltpu.make_async_copy(buf, o_hbm, wsem).wait()


@jax.jit
def pallas_standalone__grn__sampling_kernel(x: jax.Array, g: jax.Array, b: jax.Array):
    B, S, D = x.shape
    shp = (_G, B // _G, S, D)
    out = pl.pallas_call(
        _grn_kernel,
        in_specs=[pl.BlockSpec(memory_space=pl.ANY)] * 3,
        out_specs=pl.BlockSpec(memory_space=pl.ANY),
        out_shape=jax.ShapeDtypeStruct(shp, x.dtype),
        scratch_shapes=[
            pltpu.VMEM(shp, x.dtype),
            pltpu.VMEM((D,), g.dtype),
            pltpu.VMEM((D,), b.dtype),
            pltpu.VMEM((_G, D), jnp.float32),
            pltpu.VMEM((_G, D), jnp.float32),
            pltpu.VMEM((D // 128, 8 * _G, 128), jnp.float32),
            pltpu.VMEM((_G, D), jnp.float32),
            pltpu.SemaphoreType.DMA((_L,)),
            pltpu.SemaphoreType.DMA(()),
            pltpu.SemaphoreType.DMA((2,)),
        ],
        compiler_params=pltpu.CompilerParams(vmem_limit_bytes=48 * 2**20),
    )(x.reshape(shp), g, b)
    return out.reshape(B, S, D)
```

```python
import jax
import jax.numpy as jnp
import jax.experimental.pallas as pl
import jax.experimental.pallas.tpu as pltpu

_EPS = 1e-6
_LANES = 128
_SUB = 8
_G = 8
_READ_ROWS = 128
_WRITE_ROWS = 64
_WRITE_STRIDE = 4096
_DEPTH = 10
_TAIL = 3
_PART_STRIDE = 9


def _grn_kernel(x_hbm, g_hbm, b_hbm, o_hbm, buf, g_vmem, b_vmem, g_f32, b_f32, part,
                read_sems, write_sem, gb_sem, *, S, D):
    NC = D // _LANES
    RS = S * NC
    region = buf.shape[0] // _G
    rounds = region // RS
    read_steps = region // _READ_ROWS
    write_steps = _WRITE_STRIDE // _WRITE_ROWS

    early_rounds = (read_steps - _DEPTH) * _READ_ROWS // RS - 1
    late = pl.cdiv((rounds - early_rounds) * RS, _WRITE_ROWS)
    early = write_steps // 2 - late
    assert region % (_WRITE_STRIDE // 2) == 0 and early > 0

    def read_copy(k, g):
        rows = pl.ds(pl.multiple_of(g * region + k * _READ_ROWS, _READ_ROWS), _READ_ROWS)
        return pltpu.make_async_copy(
            x_hbm.at[rows], buf.at[rows], read_sems.at[jax.lax.rem(k, _DEPTH)])

    def start_reads(k):
        for g in range(_G):
            read_copy(k, g).start(priority=g % 2)

    def read_step(k, _):
        for g in range(_G):
            read_copy(k, g).wait()

        @pl.when(k + _DEPTH < read_steps)
        def _():
            start_reads(k + _DEPTH)

    def write_step(i, _):
        j = jnp.where(i < early, i,
                      jnp.where(i < 2 * early, i + late,
                                jnp.where(i < 2 * early + late, i - early, i)))
        for r in range(buf.shape[0] // _WRITE_STRIDE):
            rows = pl.ds(
                pl.multiple_of(r * _WRITE_STRIDE + j * _WRITE_ROWS, _WRITE_ROWS),
                _WRITE_ROWS)
            pltpu.make_async_copy(buf.at[rows], o_hbm.at[rows], write_sem).start()

    def sample_rows(m, g):
        return pl.ds(pl.multiple_of(g * region + m * RS, RS), RS)

    def tile(v, t):
        return v[_SUB * t:_SUB * (t + 1)]

    def lanes(c):
        return slice(_LANES * c, _LANES * (c + 1))

    def scales(m):
        for g in range(_G):
            x = buf[sample_rows(m, g)].astype(jnp.float32)
            sq = x * x
            for c in range(NC):
                p = tile(sq, c)
                for t in range(c + NC, RS // _SUB, NC):
                    p = p + tile(sq, t)
                part[c, pl.ds(_PART_STRIDE * g, _SUB), :] = p
        gx = []
        for c in range(NC):
            q = part[c, pl.ds(0, _G, stride=_PART_STRIDE), :]
            for r in range(1, _SUB):
                q = q + part[c, pl.ds(r, _G, stride=_PART_STRIDE), :]
            gx.append(jnp.sqrt(q))
        total = gx[0]
        for c in range(1, NC):
            total = total + gx[c]
        inv = 1.0 / (jnp.sum(total, axis=-1, keepdims=True) * (1.0 / D) + _EPS)
        return [g_f32[:, lanes(c)] * (gx[c] * inv) + 1.0 for c in range(NC)]

    def normalise(m, scale):
        bias = [b_f32[:, lanes(c)] for c in range(NC)]
        for g in range(_G):
            rows = sample_rows(m, g)
            x = buf[rows].astype(jnp.float32)
            sc = [jnp.broadcast_to(s[g:g + 1], (_SUB, _LANES)) for s in scale]
            y = [tile(x, t) * sc[t % NC] + bias[t % NC] for t in range(RS // _SUB)]
            buf[rows] = jnp.concatenate(y, axis=0).astype(buf.dtype)

    def steps_for(m):
        return jax.lax.div((m + 1) * RS + _READ_ROWS - 1, _READ_ROWS)

    start_reads(0)
    g_copy = pltpu.make_async_copy(g_hbm, g_vmem, gb_sem)
    b_copy = pltpu.make_async_copy(b_hbm, b_vmem, gb_sem)
    g_copy.start()
    b_copy.start()
    for k in range(1, _DEPTH):
        start_reads(k)
    g_copy.wait()
    b_copy.wait()
    g_f32[...] = jnp.broadcast_to(g_vmem[...].astype(jnp.float32).reshape(1, D), (_G, D))
    b_f32[...] = jnp.broadcast_to(b_vmem[...].astype(jnp.float32).reshape(1, D), (_SUB, D))

    first = pl.cdiv(RS, _READ_ROWS)
    jax.lax.fori_loop(0, first, read_step, None)

    def round_body(m, carry):
        k0, w0, scale = carry
        nxt = jnp.minimum(m + 1, rounds - 1)
        writing = m >= early_rounds
        k1 = steps_for(nxt)
        k1 = jnp.where(writing, jnp.maximum(k1, read_steps - _TAIL), k1)
        jax.lax.fori_loop(k0, k1, read_step, None)
        w1 = jnp.where(writing, jnp.minimum(3 + 2 * (m - early_rounds), 2 * early), 0)
        jax.lax.fori_loop(w0, w1, write_step, None)
        next_scale = scales(nxt)
        normalise(m, scale)
        return k1, w1, next_scale

    _, written, _ = jax.lax.fori_loop(0, rounds, round_body, (first, 0, scales(0)))
    jax.lax.fori_loop(written, write_steps, write_step, None)
    pltpu.make_async_copy(buf, o_hbm, write_sem).wait()


@jax.jit
def pallas_standalone__grn__sampling_kernel(x: jax.Array, g: jax.Array, b: jax.Array):
    B, S, D = x.shape
    NC = D // _LANES
    rows = B * S * NC
    assert S % (2 * _SUB) == 0 and D % _LANES == 0 and B % _G == 0
    assert rows % _WRITE_STRIDE == 0 and (rows // _G) % _READ_ROWS == 0
    tiles = x.reshape(B * S // _SUB, _SUB, NC, _LANES).transpose(0, 2, 1, 3)
    out = pl.pallas_call(
        lambda *refs: _grn_kernel(*refs, S=S, D=D),
        in_specs=[pl.BlockSpec(memory_space=pl.ANY)] * 3,
        out_specs=pl.BlockSpec(memory_space=pl.ANY),
        out_shape=jax.ShapeDtypeStruct((rows, _LANES), x.dtype),
        scratch_shapes=[
            pltpu.VMEM((rows, _LANES), x.dtype),
            pltpu.VMEM((D,), g.dtype),
            pltpu.VMEM((D,), b.dtype),
            pltpu.VMEM((_G, D), jnp.float32),
            pltpu.VMEM((_SUB, D), jnp.float32),
            pltpu.VMEM((NC, _PART_STRIDE * _G, _LANES), jnp.float32),
            pltpu.SemaphoreType.DMA((_DEPTH,)),
            pltpu.SemaphoreType.DMA(()),
            pltpu.SemaphoreType.DMA(()),
        ],
        compiler_params=pltpu.CompilerParams(
            vmem_limit_bytes=32 * 2**20,
            disable_bounds_checks=True,
            disable_semaphore_checks=True,
        ),
        name="grn",
    )(tiles.reshape(rows, _LANES), g, b)
    return out.reshape(B * S // _SUB, NC, _SUB, _LANES).transpose(0, 2, 1, 3).reshape(B, S, D)
```

```python
import functools

import jax
import jax.numpy as jnp
import jax.experimental.pallas as pl
import jax.experimental.pallas.tpu as pltpu

_EPS = 1e-6
_LANES = 128
_SUB = 8
_G = 8
_READ_ROWS = 128
_WRITE_ROWS = 64
_WRITE_STRIDE = 4096
_DEPTH = 10
_TAIL = 3
_PART_STRIDE = 9


def _grn_kernel(x_hbm, g_hbm, b_hbm, o_hbm, buf, g_vmem, b_vmem, g_f32, b_f32, part,
                write_sem, *, S, D):
    NC = D // _LANES
    RS = S * NC
    region = buf.shape[0] // _G
    rounds = region // RS
    read_steps = region // _READ_ROWS
    write_steps = _WRITE_STRIDE // _WRITE_ROWS

    early_rounds = (read_steps - _DEPTH) * _READ_ROWS // RS - 1
    late = pl.cdiv((rounds - early_rounds) * RS, _WRITE_ROWS)
    early = write_steps // 2 - late
    assert region % (_WRITE_STRIDE // 2) == 0 and early_rounds >= 0 and early > 0

    def write_step(i, _):
        j = jnp.where(i < early, i,
                      jnp.where(i < 2 * early, i + late,
                                jnp.where(i < 2 * early + late, i - early, i)))
        for r in range(buf.shape[0] // _WRITE_STRIDE):
            rows = pl.ds(
                pl.multiple_of(r * _WRITE_STRIDE + j * _WRITE_ROWS, _WRITE_ROWS),
                _WRITE_ROWS)
            pltpu.make_async_copy(buf.at[rows], o_hbm.at[rows], write_sem).start()

    def sample_rows(m, g):
        return pl.ds(pl.multiple_of(g * region + m * RS, RS), RS)

    def tile(v, t):
        return v[_SUB * t:_SUB * (t + 1)]

    def lanes(c):
        return slice(_LANES * c, _LANES * (c + 1))

    def scales(m):
        for g in range(_G):
            x = buf[sample_rows(m, g)].astype(jnp.float32)
            sq = x * x
            for c in range(NC):
                p = tile(sq, c)
                for t in range(c + NC, RS // _SUB, NC):
                    p = p + tile(sq, t)
                part[c, pl.ds(_PART_STRIDE * g, _SUB), :] = p
        gx = []
        for c in range(NC):
            q = part[c, pl.ds(0, _G, stride=_PART_STRIDE), :]
            for r in range(1, _SUB):
                q = q + part[c, pl.ds(r, _G, stride=_PART_STRIDE), :]
            gx.append(jnp.sqrt(q))
        total = gx[0]
        for c in range(1, NC):
            total = total + gx[c]
        inv = 1.0 / (jnp.sum(total, axis=-1, keepdims=True) * (1.0 / D) + _EPS)
        return [g_f32[:, lanes(c)] * (gx[c] * inv) + 1.0 for c in range(NC)]

    def normalise(m, scale):
        bias = [b_f32[:, lanes(c)] for c in range(NC)]
        for g in range(_G):
            rows = sample_rows(m, g)
            x = buf[rows].astype(jnp.float32)
            sc = [jnp.broadcast_to(s[g:g + 1], (_SUB, _LANES)) for s in scale]
            y = [tile(x, t) * sc[t % NC] + bias[t % NC] for t in range(RS // _SUB)]
            buf[rows] = jnp.concatenate(y, axis=0).astype(buf.dtype)

    def read_and_normalise(read_sems, gb_sem):
        def read_copy(k, g):
            rows = pl.ds(
                pl.multiple_of(g * region + k * _READ_ROWS, _READ_ROWS), _READ_ROWS)
            return pltpu.make_async_copy(
                x_hbm.at[rows], buf.at[rows], read_sems.at[jax.lax.rem(k, _DEPTH)])

        def start_reads(k):
            for g in range(_G):
                read_copy(k, g).start(priority=g % 2)

        def read_step(k, _):
            for g in range(_G):
                read_copy(k, g).wait()

            @pl.when(k + _DEPTH < read_steps)
            def _():
                start_reads(k + _DEPTH)

        g_copy = pltpu.make_async_copy(g_hbm, g_vmem, gb_sem)
        b_copy = pltpu.make_async_copy(b_hbm, b_vmem, gb_sem)
        g_copy.start()
        b_copy.start()
        jax.lax.fori_loop(0, _DEPTH, lambda k, _: start_reads(k), None)
        part[...] = jnp.zeros(part.shape, part.dtype)
        g_copy.wait()
        b_copy.wait()
        g_f32[...] = jnp.broadcast_to(
            g_vmem[...].astype(jnp.float32).reshape(1, D), (_G, D))
        b_f32[...] = jnp.broadcast_to(
            b_vmem[...].astype(jnp.float32).reshape(1, D), (_SUB, D))

        first = pl.cdiv(RS, _READ_ROWS)
        jax.lax.fori_loop(0, first, read_step, None)

        def round_body(m, carry):
            landed, written, scale = carry
            nxt = jnp.minimum(m + 1, rounds - 1)
            writing = m >= early_rounds
            need = jax.lax.div((nxt + 1) * RS + _READ_ROWS - 1, _READ_ROWS)
            need = jnp.where(writing, jnp.maximum(need, read_steps - _TAIL), need)
            jax.lax.fori_loop(landed, need, read_step, None)
            upto = jnp.where(
                writing, jnp.minimum(3 + 2 * (m - early_rounds), 2 * early), 0)
            jax.lax.fori_loop(written, upto, write_step, None)
            next_scale = scales(nxt)
            normalise(m, scale)
            return need, upto, next_scale

        _, written, _ = jax.lax.fori_loop(
            0, rounds, round_body, (first, 0, scales(0)))
        jax.lax.fori_loop(written, write_steps, write_step, None)

    pl.run_scoped(
        read_and_normalise,
        pltpu.SemaphoreType.DMA((_DEPTH,)),
        pltpu.SemaphoreType.DMA(()),
    )
    pltpu.make_async_copy(buf, o_hbm, write_sem).wait()


@jax.jit
def pallas_standalone__grn__sampling_kernel(x: jax.Array, g: jax.Array, b: jax.Array):
    B, S, D = x.shape
    NC = D // _LANES
    rows = B * S * NC
    assert S % (2 * _SUB) == 0 and D % _LANES == 0 and B % _G == 0
    assert rows % _WRITE_STRIDE == 0 and (rows // _G) % _READ_ROWS == 0
    tiles = x.reshape(B * S // _SUB, _SUB, NC, _LANES).transpose(0, 2, 1, 3)
    out = pl.pallas_call(
        functools.partial(_grn_kernel, S=S, D=D),
        in_specs=[pl.BlockSpec(memory_space=pl.ANY)] * 3,
        out_specs=pl.BlockSpec(memory_space=pl.ANY),
        out_shape=jax.ShapeDtypeStruct((rows, _LANES), x.dtype),
        scratch_shapes=[
            pltpu.VMEM((rows, _LANES), x.dtype),
            pltpu.VMEM((D,), g.dtype),
            pltpu.VMEM((D,), b.dtype),
            pltpu.VMEM((_G, D), jnp.float32),
            pltpu.VMEM((_SUB, D), jnp.float32),
            pltpu.VMEM((NC, _PART_STRIDE * _G + _SUB, _LANES), jnp.float32),
            pltpu.SemaphoreType.DMA(()),
        ],
        compiler_params=pltpu.CompilerParams(
            vmem_limit_bytes=32 * 2**20,
            disable_bounds_checks=True,
        ),
        name="grn",
    )(tiles.reshape(rows, _LANES), g, b)
    out = out.reshape(B * S // _SUB, NC, _SUB, _LANES).transpose(0, 2, 1, 3)
    return out.reshape(B, S, D)
```
